```python
import os as _os
_os.environ.setdefault("JAX_PLATFORMS", "cpu")
import jax
import jax.numpy as jnp

def _softmax(x, axis=-1):
    return jax.nn.softmax(x, axis=axis)
def _gelu(x):
    return jax.nn.gelu(x, approximate=True)
def _silu(x):
    return jax.nn.silu(x)
def _sigmoid(x):
    return jax.nn.sigmoid(x)
def _layernorm(x, axis=-1, eps=1e-5):
    m = jnp.mean(x, axis=axis, keepdims=True)
    v = jnp.var(x, axis=axis, keepdims=True)
    return (x - m) / jnp.sqrt(v + eps)
def _scatter_add(tgt, idx, src, axis=0):
    return tgt.at[idx].add(src)
def _segment_sum(src, seg, n):
    return jax.ops.segment_sum(src, seg, n)
class _Rng:
    def __init__(self, key):
        self._k = key
    def _next(self):
        self._k, sub = jax.random.split(self._k)
        return sub
    def normal(self, shape):
        return jax.random.normal(self._next(), shape, dtype=jnp.bfloat16)
    def randint(self, lo, hi, shape):
        return jax.random.randint(self._next(), shape, lo, hi, dtype=jnp.int32)
    def uniform(self, shape, lo=0.0, hi=1.0):
        return jax.random.uniform(self._next(), shape, jnp.bfloat16, lo, hi)
    def permutation(self, n):
        return jax.random.permutation(self._next(), n)


kernel_name = 'standalone__dcn_v2_cross__recsys'

def setup_inputs():
    _rng = _Rng(jax.random.key(int.from_bytes(__import__("os").urandom(4), "little")))
    _w = (lambda a: (lambda t: t.astype(jnp.bfloat16) if jnp.issubdtype(t.dtype, jnp.floating) else t)(jnp.asarray(a)))
    B, F, D, L = 4096, 26, 128, 6
    Din = min(F * D, 1024)
    return {
        "x0": _w((lambda *s: _rng.normal(s) * 0.05)(B, Din)),
        "ws": _w((lambda *s: _rng.normal(s) * 0.05)(L, Din, Din)),
        "bs": _w((lambda *s: _rng.normal(s) * 0.05)(L, Din)),
    }

def reference(x0, ws, bs):
    x = x0
    for l in range(ws.shape[0]):
        x = x0 * (x @ ws[l] + bs[l]) + x
    return x
```

```python
import jax
import jax.numpy as jnp
from jax import lax
import jax.experimental.pallas as pl
import jax.experimental.pallas.tpu as pltpu

F32 = jnp.float32
BF16 = jnp.bfloat16


@jax.jit
def pallas_standalone__dcn_v2_cross__recsys_kernel(
    x0: jax.Array,
    ws: jax.Array,
    bs: jax.Array,
):
    B, D = x0.shape
    L = ws.shape[0]
    tm = 512
    nt = B // tm
    c0 = (256, 256, 256, 256)
    nc0 = len(c0)
    offs0 = [sum(c0[:i]) for i in range(nc0)]

    def kernel(x0_hbm, w_hbm, b_hbm, o_hbm, xbuf, wbuf, obuf, bbuf, b32, xa,
               xsem, wsem, w0sem, osem, bsem):
        def xcopy(t):
            return pltpu.make_async_copy(
                x0_hbm.at[pl.ds(t * tm, tm)], xbuf.at[t], xsem.at[t])

        def wcopy(l):
            return pltpu.make_async_copy(w_hbm.at[l], wbuf.at[l], wsem.at[l])

        def w0copy(c):
            cs = pl.ds(offs0[c], c0[c])
            return pltpu.make_async_copy(
                w_hbm.at[0, :, cs], wbuf.at[0, :, cs], w0sem.at[c])

        def ocopy(t):
            return pltpu.make_async_copy(
                obuf.at[t], o_hbm.at[pl.ds(t * tm, tm)], osem.at[t])

        bcopy = pltpu.make_async_copy(b_hbm, bbuf, bsem.at[0])

        queue = [w0copy(c) for c in range(nc0)] + [wcopy(1)]
        bcopy.start()
        xcopy(0).start()
        queue[0].start()
        queue[1].start()
        qi = 2

        bcopy.wait()
        for l in range(L):
            b32[l] = jnp.broadcast_to(bbuf[l:l + 1, :].astype(F32), (8, D))
        xcopy(0).wait()
        for c in range(nc0):
            w0copy(c).wait()
            if qi < len(queue):
                queue[qi].start()
                qi += 1
            cs = slice(offs0[c], offs0[c] + c0[c])
            y = jnp.dot(xbuf[0], wbuf[0, :, cs], preferred_element_type=F32)
            y = y + b32[0, 0:1, cs]
            x0c = xbuf[0, :, cs].astype(F32)
            xa[0, :, cs] = (x0c * y + x0c).astype(BF16)

        def lbody(l, carry):
            wcopy(l).wait()

            @pl.when(l + 1 < L)
            def _():
                wcopy(l + 1).start()

            @pl.when(l == L - 1)
            def _():
                xcopy(1).start()

            src = (l - 1) % 2
            xb = xa[src]
            y = jnp.dot(xb, wbuf[l], preferred_element_type=F32)
            y = y + b32[l, 0:1, :]
            xa[1 - src] = (xbuf[0].astype(F32) * y + xb.astype(F32)).astype(BF16)
            return carry

        lax.fori_loop(1, L, lbody, 0)
        obuf[0] = xa[(L - 1) % 2]
        ocopy(0).start()

        def tbody(t, carry):
            xcopy(t).wait()

            @pl.when(t + 1 < nt)
            def _():
                xcopy(t + 1).start()

            xb = xbuf[t]
            for l in range(L):
                y = jnp.dot(xb, wbuf[l], preferred_element_type=F32)
                y = y + b32[l, 0:1, :]
                xb = (xbuf[t].astype(F32) * y + xb.astype(F32)).astype(BF16)
            obuf[t] = xb
            ocopy(t).start()
            return carry

        lax.fori_loop(1, nt, tbody, 0)
        for t in range(nt):
            ocopy(t).wait()

    return pl.pallas_call(
        kernel,
        in_specs=[pl.BlockSpec(memory_space=pl.ANY)] * 3,
        out_specs=pl.BlockSpec(memory_space=pl.ANY),
        out_shape=jax.ShapeDtypeStruct((B, D), BF16),
        scratch_shapes=[
            pltpu.VMEM((nt, tm, D), BF16),
            pltpu.VMEM((L, D, D), BF16),
            pltpu.VMEM((nt, tm, D), BF16),
            pltpu.VMEM((L, D), BF16),
            pltpu.VMEM((L, 8, D), F32),
            pltpu.VMEM((2, tm, D), BF16),
            pltpu.SemaphoreType.DMA((nt,)),
            pltpu.SemaphoreType.DMA((L,)),
            pltpu.SemaphoreType.DMA((nc0,)),
            pltpu.SemaphoreType.DMA((nt,)),
            pltpu.SemaphoreType.DMA((1,)),
        ],
        compiler_params=pltpu.CompilerParams(vmem_limit_bytes=100 * 1024 * 1024),
    )(x0, ws, bs)
```

```python
import jax
import jax.numpy as jnp
from jax import lax
import jax.experimental.pallas as pl
import jax.experimental.pallas.tpu as pltpu

F32 = jnp.float32
BF16 = jnp.bfloat16

_MXU = 128


def _compiler_params():
    kw = dict(vmem_limit_bytes=100 * 1024 * 1024)
    try:
        return pltpu.CompilerParams(
            disable_bounds_checks=True, disable_semaphore_checks=True, **kw)
    except TypeError:
        return pltpu.CompilerParams(**kw)


def _startup_groups(sizes, D):
    H = D // 2
    groups, pos, xk_done = [], 0, 0
    for s in sizes:
        a, b = pos, pos + s
        blocks = []
        if a % 2 == 1:
            blocks.append(((a // 2) * _MXU, _MXU, H, H))
            a += 1
        nfull = (b - a) // 2
        if nfull > 0:
            blocks.append(((a // 2) * _MXU, nfull * _MXU, 0, D))
            a += 2 * nfull
        if a < b:
            blocks.append(((a // 2) * _MXU, _MXU, 0, H))
        xk_need = ((b + 1) // 2) * _MXU
        groups.append((blocks, (xk_done, xk_need - xk_done)))
        xk_done, pos = xk_need, b
    return groups


@jax.jit
def pallas_standalone__dcn_v2_cross__recsys_kernel(
    x0: jax.Array,
    ws: jax.Array,
    bs: jax.Array,
):
    B, D = x0.shape
    L = ws.shape[0]
    assert (B, D, L) == (4096, 1024, 6), "tiling below is tuned for this shape"
    H = D // 2

    t0 = 624
    tm = 496
    ns = (B - t0) // tm
    assert t0 + ns * tm == B and t0 % 16 == 0 and tm % 16 == 0

    groups = _startup_groups((1, 2, 3, 4, 6), D)
    ng = len(groups)
    out_cols = ((0, 256), (256, 256), (512, 256), (768, 128), (896, 128))
    last_rows = ((0, 256), (256, 128), (384, 64), (448, tm - 448))

    def kernel(x0_hbm, w_hbm, b_hbm, o_hbm,
               xf, xbuf, wbuf, pbuf, obuf, acc, bbuf, b32,
               xsem, wsem, gsem, osem, rsem):

        def keep_order():
            pl.semaphore_signal(rsem, 1)
            pl.semaphore_wait(rsem, 1)

        xcopy = pltpu.make_async_copy(
            x0_hbm.at[pl.ds(t0, ns * tm)], xbuf, xsem.at[0])

        def wcopy(l):
            return pltpu.make_async_copy(w_hbm.at[l], wbuf.at[l], wsem.at[l])

        def gcopies(g):
            blocks, (xk0, xkn) = groups[g]
            cps = []
            if xkn > 0:
                kk = pl.ds(xk0, xkn)
                cps.append(pltpu.make_async_copy(
                    x0_hbm.at[pl.ds(0, t0), kk], xf.at[:, kk], gsem.at[g]))
            for (k0, kn, n0, nn) in blocks:
                kk, nn_ = pl.ds(k0, kn), pl.ds(n0, nn)
                cps.append(pltpu.make_async_copy(
                    w_hbm.at[0, kk, nn_], wbuf.at[0, kk, nn_], gsem.at[g]))
            if g == ng - 1:
                cps.append(pltpu.make_async_copy(b_hbm, bbuf, gsem.at[g]))
            return cps

        def dot(a, b):
            return jnp.dot(a, b, preferred_element_type=F32)

        def fast_start_dot(xb, wl):
            ya = dot(xb[:, :_MXU], wl[:_MXU, :H])
            ya = dot(xb[:, _MXU:], wl[_MXU:, :H]) + ya
            yb = dot(xb, wl[:, H:])
            return jnp.concatenate([ya, yb], axis=1)

        def first_tile():
            for g in range(ng):
                for cp in gcopies(g):
                    cp.start()
                keep_order()
            for l in range(1, L):
                wcopy(l).start()
                keep_order()
            xcopy.start()

            inited = [False, False]
            for g in range(ng):
                for cp in gcopies(g):
                    cp.wait()
                last = g == ng - 1
                if last:
                    for l in range(L):
                        b32[l] = jnp.broadcast_to(
                            bbuf[l:l + 1, :].astype(F32), (8, D))
                for hh in range(2):
                    kr = [(k0, k0 + kn) for (k0, kn, n0, nn) in groups[g][0]
                          if n0 <= hh * H < n0 + nn]
                    if not kr:
                        continue
                    k0, k1 = min(k for k, _ in kr), max(k for _, k in kr)
                    cs = slice(hh * H, (hh + 1) * H)
                    p = dot(xf[:, k0:k1], wbuf[0, k0:k1, cs])
                    if last:
                        y = acc[:, cs] + p + bbuf[0:1, cs].astype(F32)
                        x0c = xf[:, cs].astype(F32)
                        pbuf[0, :, cs] = (x0c * y + x0c).astype(BF16)
                    elif inited[hh]:
                        acc[:, cs] += p
                    else:
                        acc[:, cs] = p
                        inited[hh] = True

            def layer(l, carry):
                wcopy(l).wait()
                dst = l & 1
                src = 1 - dst
                xb = pbuf[src]
                y = fast_start_dot(xb, wbuf.at[l]) + b32[l, 0:1, :]
                pbuf[dst] = (xf[...].astype(F32) * y
                             + xb.astype(F32)).astype(BF16)
                return carry

            lax.fori_loop(1, L, layer, 0)
            pltpu.make_async_copy(
                pbuf.at[(L - 1) % 2], o_hbm.at[pl.ds(0, t0)], osem.at[0]).start()
            xcopy.wait()

        def steady_tile(t):
            r0 = pl.multiple_of(t * tm, 16)
            rs = pl.ds(r0, tm)
            xb = xbuf[rs, :]
            for l in range(L - 1):
                y = fast_start_dot(xb, wbuf.at[l]) if l == 0 else dot(xb, wbuf[l])
                y = y + b32[l, 0:1, :]
                xb = (xbuf[rs, :].astype(F32) * y + xb.astype(F32)).astype(BF16)
            x = xb.astype(F32)
            for c, (c0, cn) in enumerate(out_cols):
                cs, cd = slice(c0, c0 + cn), pl.ds(c0, cn)
                y = dot(xb, wbuf[L - 1, :, cs]) + b32[L - 1, 0:1, cs]
                res = (xbuf[rs, cs].astype(F32) * y + x[:, cs]).astype(BF16)
                pieces = last_rows if c == len(out_cols) - 1 else ((0, tm),)
                for (q0, qn) in pieces:
                    rq = pl.ds(pl.multiple_of(r0 + q0, 16), qn)
                    obuf[rq, cs] = res[q0:q0 + qn]
                    pltpu.make_async_copy(
                        obuf.at[rq, cd],
                        o_hbm.at[pl.ds(t0 + r0 + q0, qn), cd],
                        osem.at[0]).start()

        def step(t, carry):
            @pl.when(t == 0)
            def _():
                first_tile()

            steady_tile(t)
            return carry

        lax.fori_loop(0, ns, step, 0)
        pltpu.make_async_copy(o_hbm, o_hbm, osem.at[0]).wait()

    return pl.pallas_call(
        kernel,
        in_specs=[pl.BlockSpec(memory_space=pl.ANY)] * 3,
        out_specs=pl.BlockSpec(memory_space=pl.ANY),
        out_shape=jax.ShapeDtypeStruct((B, D), BF16),
        scratch_shapes=[
            pltpu.VMEM((t0, D), BF16),
            pltpu.VMEM((ns * tm, D), BF16),
            pltpu.VMEM((L, D, D), BF16),
            pltpu.VMEM((2, t0, D), BF16),
            pltpu.VMEM((ns * tm, D), BF16),
            pltpu.VMEM((t0, D), F32),
            pltpu.VMEM((L, D), BF16),
            pltpu.VMEM((L, 8, D), F32),
            pltpu.SemaphoreType.DMA((1,)),
            pltpu.SemaphoreType.DMA((L,)),
            pltpu.SemaphoreType.DMA((ng,)),
            pltpu.SemaphoreType.DMA((1,)),
            pltpu.SemaphoreType.REGULAR,
        ],
        compiler_params=_compiler_params(),
    )(x0, ws, bs)
```

```python
import jax
import jax.numpy as jnp
from jax import lax
import jax.experimental.pallas as pl
import jax.experimental.pallas.tpu as pltpu

F32 = jnp.float32
BF16 = jnp.bfloat16

_MXU = 128


def _compiler_params():
    kw = dict(vmem_limit_bytes=100 * 1024 * 1024)
    try:
        return pltpu.CompilerParams(
            disable_bounds_checks=True, disable_semaphore_checks=True, **kw)
    except TypeError:
        return pltpu.CompilerParams(**kw)


def _startup_groups(sizes, D):
    H = D // 2
    assert sum(sizes) == 2 * (D // _MXU)
    groups, pos, xk_done = [], 0, 0
    for size in sizes:
        a, b = pos, pos + size
        blocks = []
        if a % 2 == 1:
            blocks.append(((a // 2) * _MXU, _MXU, H, H))
            a += 1
        nfull = (b - a) // 2
        if nfull > 0:
            blocks.append(((a // 2) * _MXU, nfull * _MXU, 0, D))
            a += 2 * nfull
        if a < b:
            blocks.append(((a // 2) * _MXU, _MXU, 0, H))
        xk_need = ((b + 1) // 2) * _MXU
        groups.append((blocks, (xk_done, xk_need - xk_done)))
        xk_done, pos = xk_need, b
    return groups


@jax.jit
def pallas_standalone__dcn_v2_cross__recsys_kernel(
    x0: jax.Array,
    ws: jax.Array,
    bs: jax.Array,
):
    B, D = x0.shape
    L = ws.shape[0]
    assert (B, D, L) == (4096, 1024, 6), "tiling below is tuned for this shape"
    H = D // 2

    nt = 8
    s = 80
    J = 3
    t0 = nt * s
    tm = B // nt - s
    assert t0 + nt * tm == B and s % 16 == 0 and tm % 16 == 0

    groups = _startup_groups((1, 2, 3, 4, 6), D)
    ng = len(groups)
    out_cols = ((0, 256), (256, 256), (512, 256), (768, 128), (896, 128))
    last_rows = ((0, 192), (192, 128), (320, 64), (384, tm - 384))

    def kernel(x0_hbm, w_hbm, b_hbm, o_hbm,
               xf, xbuf, wbuf, pbuf, obuf, acc, bbuf, b32,
               xsem, wsem, gsem, osem, rsem):

        def keep_order():
            pl.semaphore_signal(rsem, 1)
            pl.semaphore_wait(rsem, 1)

        def xcopy(t):
            return pltpu.make_async_copy(
                x0_hbm.at[pl.ds(t0 + t * tm, tm)], xbuf.at[t], xsem.at[t])

        def wcopy(l):
            return pltpu.make_async_copy(w_hbm.at[l], wbuf.at[l], wsem.at[l])

        wrest = pltpu.make_async_copy(
            w_hbm.at[pl.ds(J, L - J)], wbuf.at[pl.ds(J, L - J)], wsem.at[0])

        def gcopies(g):
            blocks, (xk0, xkn) = groups[g]
            cps = []
            if xkn > 0:
                kk = pl.ds(xk0, xkn)
                cps.append(pltpu.make_async_copy(
                    x0_hbm.at[pl.ds(0, t0), kk], xf.at[:, kk], gsem.at[g]))
            for (k0, kn, n0, nn) in blocks:
                kk, nn_ = pl.ds(k0, kn), pl.ds(n0, nn)
                cps.append(pltpu.make_async_copy(
                    w_hbm.at[0, kk, nn_], wbuf.at[0, kk, nn_], gsem.at[g]))
            if g == ng - 1:
                cps.append(pltpu.make_async_copy(b_hbm, bbuf, gsem.at[g]))
            return cps

        def dot(a, b):
            return jnp.dot(a, b, preferred_element_type=F32)

        def fast_start_dot(xb, wl):
            ya = dot(xb[:, :_MXU], wl[:_MXU, :H])
            ya = dot(xb[:, _MXU:], wl[_MXU:, :H]) + ya
            yb = dot(xb, wl[:, H:])
            return jnp.concatenate([ya, yb], axis=1)

        def startup():
            for g in range(ng):
                for cp in gcopies(g):
                    cp.start()
                keep_order()
            for l in range(1, J):
                wcopy(l).start()
                keep_order()
            wrest.start()
            keep_order()
            for t in range(nt):
                xcopy(t).start()
                keep_order()

            inited = [False, False]
            for g in range(ng):
                for cp in gcopies(g):
                    cp.wait()
                last = g == ng - 1
                if last:
                    for l in range(L):
                        b32[l] = jnp.broadcast_to(
                            bbuf[l:l + 1, :].astype(F32), (8, D))
                for hh in range(2):
                    kr = [(k0, k0 + kn) for (k0, kn, n0, nn) in groups[g][0]
                          if n0 <= hh * H < n0 + nn]
                    if not kr:
                        continue
                    k0, k1 = min(k for k, _ in kr), max(k for _, k in kr)
                    cs = slice(hh * H, (hh + 1) * H)
                    p = dot(xf[:, k0:k1], wbuf[0, k0:k1, cs])
                    if last:
                        y = acc[:, cs] + p + bbuf[0:1, cs].astype(F32)
                        x0c = xf[:, cs].astype(F32)
                        pbuf[0, :, cs] = (x0c * y + x0c).astype(BF16)
                    elif inited[hh]:
                        acc[:, cs] += p
                    else:
                        acc[:, cs] = p
                        inited[hh] = True

            def layer(l, carry):
                wcopy(l).wait()
                dst = l & 1
                src = 1 - dst
                xb = pbuf[src]
                y = fast_start_dot(xb, wbuf.at[l]) + b32[l, 0:1, :]
                pbuf[dst] = (xf[...].astype(F32) * y
                             + xb.astype(F32)).astype(BF16)
                return carry

            lax.fori_loop(1, J, layer, 0)
            wrest.wait()

        def steady(t):
            xcopy(t).wait()
            xb = xbuf[t]
            for l in range(J):
                y = fast_start_dot(xb, wbuf.at[l]) if l == 0 else dot(xb, wbuf[l])
                y = y + b32[l, 0:1, :]
                xb = (xbuf[t].astype(F32) * y + xb.astype(F32)).astype(BF16)

            es = pl.ds(pl.multiple_of(t * s, 16), s)
            xb = jnp.concatenate([pbuf[(J - 1) % 2, es, :], xb], axis=0)

            def x0_f32(cs):
                return jnp.concatenate(
                    [xf[es, cs].astype(F32), xbuf[t, :, cs].astype(F32)], axis=0)

            for l in range(J, L - 1):
                y = dot(xb, wbuf[l]) + b32[l, 0:1, :]
                xb = (x0_f32(slice(None)) * y + xb.astype(F32)).astype(BF16)

            x = xb.astype(F32)
            r0 = pl.multiple_of(t0 + t * tm, 16)
            for c, (c0, cn) in enumerate(out_cols):
                cs, cd = slice(c0, c0 + cn), pl.ds(c0, cn)
                y = dot(xb, wbuf[L - 1, :, cs]) + b32[L - 1, 0:1, cs]
                res = (x0_f32(cs) * y + x[:, cs]).astype(BF16)
                obuf[t, 0:s, cs] = res[0:s]
                pltpu.make_async_copy(
                    obuf.at[t, pl.ds(0, s), cd], o_hbm.at[es, cd],
                    osem.at[0]).start()
                pieces = last_rows if c == len(out_cols) - 1 else ((0, tm),)
                for (q0, qn) in pieces:
                    obuf[t, s + q0:s + q0 + qn, cs] = res[s + q0:s + q0 + qn]
                    pltpu.make_async_copy(
                        obuf.at[t, pl.ds(s + q0, qn), cd],
                        o_hbm.at[pl.ds(r0 + q0, qn), cd],
                        osem.at[0]).start()

        def step(t, carry):
            @pl.when(t == 0)
            def _():
                startup()

            steady(t)
            return carry

        lax.fori_loop(0, nt, step, 0)
        pltpu.make_async_copy(o_hbm, o_hbm, osem.at[0]).wait()

    return pl.pallas_call(
        kernel,
        in_specs=[pl.BlockSpec(memory_space=pl.ANY)] * 3,
        out_specs=pl.BlockSpec(memory_space=pl.ANY),
        out_shape=jax.ShapeDtypeStruct((B, D), BF16),
        scratch_shapes=[
            pltpu.VMEM((t0, D), BF16),
            pltpu.VMEM((nt, tm, D), BF16),
            pltpu.VMEM((L, D, D), BF16),
            pltpu.VMEM((2, t0, D), BF16),
            pltpu.VMEM((nt, s + tm, D), BF16),
            pltpu.VMEM((t0, D), F32),
            pltpu.VMEM((L, D), BF16),
            pltpu.VMEM((L, 8, D), F32),
            pltpu.SemaphoreType.DMA((nt,)),
            pltpu.SemaphoreType.DMA((J,)),
            pltpu.SemaphoreType.DMA((ng,)),
            pltpu.SemaphoreType.DMA((1,)),
            pltpu.SemaphoreType.REGULAR,
        ],
        compiler_params=_compiler_params(),
    )(x0, ws, bs)
```
